```python
import os as _os
_os.environ.setdefault("JAX_PLATFORMS", "cpu")
import jax
import jax.numpy as jnp

def _softmax(x, axis=-1):
    return jax.nn.softmax(x, axis=axis)
def _gelu(x):
    return jax.nn.gelu(x, approximate=True)
def _silu(x):
    return jax.nn.silu(x)
def _sigmoid(x):
    return jax.nn.sigmoid(x)
def _layernorm(x, axis=-1, eps=1e-5):
    m = jnp.mean(x, axis=axis, keepdims=True)
    v = jnp.var(x, axis=axis, keepdims=True)
    return (x - m) / jnp.sqrt(v + eps)
def _scatter_add(tgt, idx, src, axis=0):
    return tgt.at[idx].add(src)
def _segment_sum(src, seg, n):
    return jax.ops.segment_sum(src, seg, n)
class _Rng:
    def __init__(self, key):
        self._k = key
    def _next(self):
        self._k, sub = jax.random.split(self._k)
        return sub
    def normal(self, shape):
        return jax.random.normal(self._next(), shape, dtype=jnp.bfloat16)
    def randint(self, lo, hi, shape):
        return jax.random.randint(self._next(), shape, lo, hi, dtype=jnp.int32)
    def uniform(self, shape, lo=0.0, hi=1.0):
        return jax.random.uniform(self._next(), shape, jnp.bfloat16, lo, hi)
    def permutation(self, n):
        return jax.random.permutation(self._next(), n)


kernel_name = 'sequential_preLN__softmax_full_mha__dense_activation_squared_relu__prompt'

def setup_inputs():
    _rng = _Rng(jax.random.key(int.from_bytes(__import__("os").urandom(4), "little")))
    _w = (lambda a: (lambda t: t.astype(jnp.bfloat16) if jnp.issubdtype(t.dtype, jnp.floating) else t)(jnp.asarray(a)))
    def _A_setup():
        B, S, D = 1, 2048, 640
        return {
            "x": _w((lambda *s: _rng.normal(s) * 0.05)(B, S, D)),
            "wqkv": _w((lambda *s: _rng.normal(s) * 0.05)(D, 3 * D)),
            "wo": _w((lambda *s: _rng.normal(s) * 0.05)(D, D)),
        }
    _A_in = _A_setup()

    def _B_setup():
        B, S, D, F = 1, 2048, 640, 1536
        return {
            "x": _w((lambda *s: _rng.normal(s) * 0.05)(B, S, D)),
            "w1": _w((lambda *s: _rng.normal(s) * 0.05)(D, F)),
            "b1": _w((lambda *s: _rng.normal(s) * 0.05)(F)),
            "w2": _w((lambda *s: _rng.normal(s) * 0.05)(F, D)),
            "b2": _w((lambda *s: _rng.normal(s) * 0.05)(D)),
        }
    _B_in = _B_setup()

    return {
        "A_x": _A_in["x"],
        "A_wqkv": _A_in["wqkv"],
        "A_wo": _A_in["wo"],
        "B_x": _B_in["x"],
        "B_w1": _B_in["w1"],
        "B_b1": _B_in["b1"],
        "B_w2": _B_in["w2"],
        "B_b2": _B_in["b2"],
    }

def reference(A_x, A_wqkv, A_wo, B_x, B_w1, B_b1, B_w2, B_b2):
    def _A_ref(x, wqkv, wo):
        B, S, D = x.shape
        H = 32; Dh = D // H
        qkv = (lambda x, *d: x.transpose(*d))((x @ wqkv).reshape(B, S, 3, H, Dh), 2, 0, 3, 1, 4)
        q, k, v = qkv[0], qkv[1], qkv[2]
        scale = Dh ** -0.5
        scores = jnp.einsum("bhqd,bhkd->bhqk", q, k) * scale
        p = _softmax(scores, axis=-1)
        o = jnp.einsum("bhqk,bhkd->bhqd", p, v)
        return (lambda x, *d: x.transpose(*d))(o, 0, 2, 1, 3).reshape(B, S, D) @ wo

    def _B_ref(x, w1, b1, w2, b2):
        h = jnp.einsum("bsd,df->bsf", x, w1) + b1
        zero = jnp.zeros_like(h)
        r = jnp.where(h > zero, h, zero)
        h = r * r
        out = jnp.einsum("bsf,fd->bsd", h, w2) + b2
        return out

    x = A_x
    h = x + _A_ref(_layernorm(x, axis=-1), A_wqkv, A_wo)
    h2 = h + _B_ref(_layernorm(h, axis=-1), B_w1, B_b1, B_w2, B_b2)
    return h2
```

```python
import functools
import math

import jax
import jax.numpy as jnp
from jax import lax
import jax.experimental.pallas as pl
import jax.experimental.pallas.tpu as pltpu

F32 = jnp.float32
BF16 = jnp.bfloat16
U32 = jnp.uint32

S, D, H, DH, F = 2048, 640, 32, 20, 1536
L = 128
QSCALE = DH ** -0.5 * math.log2(math.e)

TB = 256
NB = S // TB
RC = 16
KS = 4 * L
NQ = 14 * L

BQ = 512
NU, NC = S // BQ, BQ // L
SK = S // 2
NV = 128
NG = NV // 8
NCH = SK // L
CH = (SK - NV) // NCH
AHEAD = 2
NSLAB = D // L
CROSS = [h for h in range(H) if DH * h // L != (DH * h + DH - 1) // L]
NSL = NSLAB + len(CROSS)

PHASE = (0, 0, 4, 0, 0, 0, 0, 0)
LAG = (29, 27, 30, 30, 30, 30, 30, 30)
COLUMN = (1, 1, 1, 1, 1, 1, 1, 0)

KSTRIDE = 22
KSPARE = 511
KJOBS = [(g, d) for g in range(NG) for d in range(0, DH, 2)]
KPLAN = [[jobs[u * len(jobs) // NU:(u + 1) * len(jobs) // NU] for u in range(NU)]
         for jobs in (KJOBS + [None] * 10, KJOBS + [None] * 15)]
KGROUPS = [[sorted({job[0] for job in part if job}) for part in plan] for plan in KPLAN]
KSLOTS = 6
assert all(len(groups) <= KSLOTS for plan in KGROUPS for groups in plan)

G_PACE = DH * NC
G_K = G_PACE + 1 + 0
G_Q = G_K + H * 2 * KSLOTS + 0
G_W = G_Q + H * NC * 3 + 2
G_END = -(-(G_W + NSL * NC * 8) // 4) * 4

LEFT = (((0, 1), (3, 1)), ((2, 1), (3, 1)), ((0, 1),), ((3, 1),), ((0, 1), (1, 1)),
        ((2, 1), (0, -1)), ((1, 1), (3, -1)))
RIGHT = (((0, 1), (3, 1)), ((0, 1),), ((1, 1), (3, -1)), ((2, 1), (0, -1)), ((3, 1),),
         ((0, 1), (1, 1)), ((2, 1), (3, 1)))
RESULT = (((0, 1), (3, 1), (4, -1), (6, 1)), ((2, 1), (4, 1)), ((1, 1), (3, 1)),
          ((0, 1), (1, -1), (2, 1), (5, 1)))


def mm(a, b):
    return lax.dot_general(a, b, (((1,), (0,)), ((), ())), preferred_element_type=F32)


def combine(terms, get):
    total = get(terms[0][0])
    for i, sign in terms[1:]:
        total = total + get(i) if sign > 0 else total - get(i)
    return total


def cut(x):
    return lambda r, c: x[r:r + RC, c:c + L]


def assemble(tile, m, n):
    return jnp.concatenate([jnp.concatenate([tile(r, c) for c in range(0, n, L)], axis=1)
                            for r in range(0, m, RC)], axis=0)


def operands(tile, m, k, table):
    sums = {}
    for r in range(0, m // 2, RC):
        for c in range(0, k // 2, L):
            quarters = [tile(i * (m // 2) + r, j * (k // 2) + c) for i in range(2) for j in range(2)]
            sums[r, c] = [combine(terms, lambda q: quarters[q]) for terms in table]
    return [assemble(lambda r, c: sums[r, c][i], m // 2, k // 2).astype(BF16) for i in range(7)]


def store_right(dst, src, k, n):
    tile = lambda r, c: src[pl.ds(r, RC), pl.ds(c, L)].astype(F32)
    for i, operand in enumerate(operands(tile, k, n, RIGHT)):
        dst[pl.ds(i * k // 4, k // 4), :] = pltpu.bitcast(operand, U32)


def strassen(left, right, order, extra):
    rows = right.shape[0] // 7
    products = {}
    for step in order:
        if step == "x":
            extra()
        else:
            i = int(step)
            products[i] = mm(left[i], pltpu.bitcast(right[pl.ds(i * rows, rows), :], BF16))
    m, n = products[0].shape

    @functools.cache
    def quarters(r, c):
        pieces = [products[i][r:r + RC, c:c + L] for i in range(7)]
        return [combine(terms, lambda i: pieces[i]) for terms in RESULT]
    return lambda r, c: quarters(r % m, c % n)[2 * (r // m) + c // n]


def layernorm(tile):
    @functools.cache
    def rows(r):
        x = [tile(r, c) for c in range(0, D, L)]
        mean = jnp.sum(functools.reduce(jnp.add, x), axis=-1, keepdims=True) * (1.0 / D)
        x = [t - mean for t in x]
        var = jnp.sum(functools.reduce(jnp.add, [t * t for t in x]), axis=-1, keepdims=True) * (1.0 / D)
        scale = lax.rsqrt(var + 1e-5)
        return [t * scale for t in x]
    return lambda r, c: rows(r)[c // L]


def spread(*lists):
    at = [(lo + (hi - lo) * (i + .5) / len(jobs), n, i)
          for n, (jobs, lo, hi) in enumerate(lists) for i in range(len(jobs))]
    return [lists[n][0][i] for _, n, i in sorted(at)]


class Table:
    def __init__(self, ref):
        self.ref = ref

    def rows(self, i):
        return pl.ds(8 * i if isinstance(i, int) else pl.multiple_of(8 * i, 8), 8)

    def __getitem__(self, i):
        return self.ref[self.rows(i), :]

    def __setitem__(self, i, value):
        self.ref[self.rows(i), :] = value


def kernel(x_hbm, wqkv_hbm, wo_hbm, w1_hbm, b1_hbm, w2_hbm, b2_hbm, out_hbm,
           x_s, wqkv_s, wo_s, w1_s, w2_s, out_s, rq_s, ro_s, r1_s, r2_s, o_s,
           k_s, vt_s, w_s, g0_s, g1_s, g2_s, g3_s, kb0_s, kb1_s, p0_s, p1_s, ot_s, acc_s,
           b1_s, b2_s, spare_s, in_sem, out_sem):
    g_s = [Table(g) for g in (g0_s, g1_s, g2_s, g3_s)]
    kb_s = (kb0_s, kb1_s)
    p_s = (p0_s, p1_s)

    def fetch(src, dst, i):
        return pltpu.make_async_copy(src, dst, in_sem.at[i])
    x_cp = [fetch(x_hbm.at[pl.ds(b * TB, TB)], x_s.at[pl.ds(b * TB, TB)], 7 + b) for b in range(NB)]
    w_tail_cp = fetch(wqkv_hbm.at[pl.ds(KS, D - KS)], wqkv_s.at[pl.ds(KS, D - KS)], 0)
    w_main_cp = fetch(wqkv_hbm.at[pl.ds(0, KS)], wqkv_s.at[pl.ds(0, KS)], 1)
    later_cp = [fetch(wo_hbm, wo_s, 2), fetch(w1_hbm, w1_s, 3), fetch(w2_hbm, w2_s, 4),
                fetch(b1_hbm, b1_s, 5), fetch(b2_hbm, b2_s, 6)]
    first = 3

    x_cp[0].start()
    w_tail_cp.start()
    for cp in x_cp[1:first]:
        cp.start()
    for p in p_s:
        p[...] = jnp.zeros(p.shape, U32)
    w_main_cp.start()
    spare_s[0] = G_PACE
    spare_s[1] = KSPARE
    spare_s[2] = NU

    sub = lax.broadcasted_iota(jnp.int32, (8, TB), 0)
    lane = lax.broadcasted_iota(jnp.int32, (TB // 2, L), 1)
    word = lax.broadcasted_iota(jnp.int32, (L // 2, TB), 0)

    def normed(b):
        tile = layernorm(lambda r, c: x_s[pl.ds(b * TB + r, RC), pl.ds(c, L)].astype(F32))
        for r in range(0, TB, RC):
            tile(r, 0)
        return tile

    def tail_product(tile):
        return cut(mm(assemble(lambda r, c: tile(r, KS), TB, L).astype(BF16), wqkv_s[KS:, :NQ]))

    xn, tail = {}, {}
    for cp in x_cp[:first] + [w_tail_cp]:
        cp.wait()
    for b in range(first):
        xn[b] = normed(b)
        tail[b] = tail_product(xn[b])
    for cp in x_cp[first:]:
        cp.start()
    w_main_cp.wait()

    for b in range(NB):
        if b == 0:
            store_right(rq_s, wqkv_s, KS, NQ)

        def rest():
            if b not in tail:
                tail[b] = tail_product(xn[b])
        main = strassen(operands(xn[b], TB, KS, LEFT), rq_s, "x1432056", rest)
        qkv = lambda r, c: main(r, c) + tail[b](r, c)
        last = cut(mm(assemble(xn[b], TB, D).astype(BF16), wqkv_s[:, NQ:]))
        if b == 0:
            for cp in x_cp[first:]:
                cp.wait()
            for cp in later_cp:
                cp.start()
        for i in range(b + 1, min(b + 3, NB)):
            if i not in xn:
                xn[i] = normed(i)

        k = assemble(lambda r, c: qkv(r, D + c), TB, D)
        packed = pltpu.bitcast(k.astype(BF16), F32)
        slabs = [packed[:, j * L:(j + 1) * L] for j in range(NSLAB)]
        for h in CROSS:
            j = DH * h // L
            slabs.append(jnp.where(lane >= DH * h % L, slabs[j], slabs[j + 1]))
        for r in range(0, TB // 2, 8):
            for j, slab in enumerate(slabs):
                k_s[j, pl.ds(b * TB // 2 + r, 8), :] = slab[r:r + 8]
        for half in range(2):
            for g in range(NG):
                r = half * SK + 8 * g - b * TB
                for h in range(H if 0 <= r < TB else 0):
                    j, off = divmod(DH * h, L)
                    kk = k[r:r + 8, j * L:(j + 1) * L]
                    if h in CROSS:
                        kk = jnp.where(lane[:8] >= off, kk, k[r:r + 8, (j + 1) * L:(j + 2) * L])
                    kk = pltpu.roll(kk, L - off, 1) if off else kk
                    for u in range(NU):
                        if g in KGROUPS[half][u]:
                            g_s[u][G_K + (h * 2 + half) * KSLOTS + KGROUPS[half][u].index(g)] = kk

        qt = assemble(lambda r, c: qkv(r, c) * QSCALE, TB, D).T
        qt4 = pltpu.roll(qt, D - 4, 0)
        tiles = [divmod(b * TB // L + c, NC) for c in range(TB // L)]
        for h in range(H):
            src, r = (qt4, DH * h - 4) if h & 1 else (qt, DH * h)
            for c, (u, col) in enumerate(tiles):
                for i in range(3):
                    g_s[(u + 1) % NU][G_Q + (h * NC + col) * 3 + i] = src[r + 8 * i:r + 8 * i + 8, c * L:(c + 1) * L]
        packed = pltpu.bitcast(qt.astype(BF16), F32)
        slabs = [packed[j * L // 2:(j + 1) * L // 2] for j in range(NSLAB)]
        for h in CROSS:
            j = DH * h // L
            slabs.append(jnp.where(word >= DH * h % L // 2, slabs[j], slabs[j + 1]))
        for j, slab in enumerate(slabs):
            for c, (u, col) in enumerate(tiles):
                for i in range(8):
                    g_s[(u + 1) % NU][G_W + (j * NC + col) * 8 + i] = slab[8 * i:8 * i + 8, c * L:(c + 1) * L]

        vt = assemble(lambda r, c: qkv(r, 2 * D + c) if 2 * D + c < NQ else last(r, 0), TB, D).T
        rows = []
        for h in range(0, H, 2):
            r = DH * h
            mid = vt[r + 16:r + 24]
            rows += [jnp.concatenate([vt[r:r + 16], jnp.where(sub < 4, mid, 1.0)], axis=0),
                     jnp.concatenate([jnp.where(sub < 4, 1.0, mid), vt[r + 24:r + 40]], axis=0)]
        for h in range(H):
            vt_s[h, :, pl.ds(b * TB, TB)] = rows[h]

    sub8 = lax.broadcasted_iota(jnp.int32, (8, L), 0)

    def slab_of(h):
        j = (h * DH) >> 7
        for i, crossing in enumerate(CROSS):
            j = jnp.where(h == crossing, NSLAB + i, j)
        return j

    def w_tile(h, slab, u, c, i):
        rel = (sub8 + (8 * i - ((h * (DH // 2)) & 63))) & 63
        return jnp.where(rel < DH // 2, g_s[(u + 1) % NU][G_W + (slab * NC + c) * 8 + i], 0.0)

    def w_jobs(h, u):
        slab = slab_of(h)

        def job(c, i):
            w_s[u, pl.ds(8 * i, 8), pl.ds(c * L, L)] = w_tile(h, slab, u, c, i)
        return [functools.partial(job, c, i) for c in range(NC) for i in range(8)]

    def q_jobs(h, u):
        rows = {}

        def load(i, c):
            rows[i, c] = g_s[(u + 1) % NU][G_Q + (h * NC + c) * 3 + i]

        def job(c, d):
            g_s[u][d * NC + c] = jnp.broadcast_to(rows[d // 8, c][d % 8:d % 8 + 1], (8, L))
        jobs = []
        for c in range(NC):
            for d in range(DH):
                if d % 2 == 0:
                    jobs.append(functools.partial(load, d // 8, c))
                jobs.append(functools.partial(job, c, d))
        return jobs

    def k_jobs(h, half, u):
        def job(g, d):
            kk = g_s[u][G_K + (h * 2 + half) * KSLOTS + KGROUPS[half][u].index(g)]
            kk = pltpu.roll(kk, L - d, 1) if d else kk
            for i in range(2):
                kb_s[half][g * KSTRIDE + d + i] = jnp.broadcast_to(kk[:, i:i + 1], (8, L))
        return [functools.partial(job, *j) if j else (lambda: None) for j in KPLAN[half][u]]

    def store_exp(half, key, cols, scores):
        p = jnp.exp2(scores).astype(BF16)
        p_s[half][pl.ds(key // 2, scores.shape[0] // 2), cols] = pltpu.bitcast(p, U32)

    segments = [(half, u) for half in range(2) for u in range(NU)]
    steps = [(half, u, j) for half, u in segments for j in range(NCH)]

    def probabilities(i):
        half, u, j = steps[i]
        return pltpu.bitcast(p_s[half][pl.ds(j * L // 2, L // 2), pl.ds(u * BQ, BQ)], BF16)

    def weigh_values(i, head, slot, p=None):
        half, u, j = steps[i]
        cols = pl.ds(u * BQ, BQ)
        p = probabilities(i) if p is None else p
        r = mm(vt_s[head, :, pl.ds(half * SK + j * L, L)], p)
        if j:
            r = acc_s[0:24, :] + r
        elif half:
            r = ot_s[slot, :, cols] + r
        if j == NCH - 1:
            ot_s[slot, :, cols] = r
        else:
            acc_s[0:24, :] = r

    def one_head(h, carry):
        slab = slab_of(h)
        following = jnp.minimum(h + 1, H - 1)
        previous = jnp.maximum(h - 1, 0)
        slot = jnp.where(h > 0, h - 1, H)

        jobs = []
        for n, (half, u) in enumerate(segments):
            head = (h, following)[half]
            lists = [(k_jobs(head, 1 - half, u), 0, 1)]
            if n in (5, 6, 7, 0):
                wj = w_jobs(head, (u - 1) % NU)
                if n == 0:
                    def keep_order():
                        w_s[spare_s[2] & 7, 0:8, 0:L] = jnp.zeros((8, L), F32)
                    wj.append(keep_order)
                lists += [(wj, 0, .07), (q_jobs(head, (u - 1) % NU), 0, .5)]
            jobs.append(spread(*lists, ([lambda: None] * 64, 0, 1)))

        pace = spare_s[0] & 127
        opening = [probabilities(i) for i in range(AHEAD)]
        for i in range(AHEAD):
            weigh_values(i, previous, slot, opening[i])
        held = []
        scores = []
        per_segment = (SK - NV) // 8
        features = NG // 2 * DH
        sums = [None, None]
        for i, (half, u, j) in enumerate(steps):
            cols = pl.ds(u * BQ, BQ)
            n = i // NCH
            if j == 0 and n == NU:
                kb1_s[spare_s[1] & 511] = jnp.zeros((8, L), F32)
            key = NV + j * CH
            s = mm(pltpu.bitcast(k_s[slab, pl.ds((half * SK + key) // 2, CH // 2), :], BF16),
                   pltpu.bitcast(w_s[u], BF16))
            scores += [s[r:r + 8, COLUMN[n] * L:(COLUMN[n] + 1) * L] for r in range(0, CH, 8)]
            store_exp(half, key, cols, s)

            e0, e1 = j * features // NCH, (j + 1) * features // NCH
            todo = jobs[n][j * len(jobs[n]) // NCH:(j + 1) * len(jobs[n]) // NCH]
            done = 0
            for e in range(e0, e1):
                pair, d = divmod(e, DH)
                t = (n * features + e) * 4 + PHASE[n]
                recent = min(n * per_segment + e * per_segment // features - LAG[n], len(scores) - 1)
                if t // 10 != (t - 4) // 10 and recent >= 0:
                    g_s[u][pace] = scores[recent]
                while done < len(todo) and done * (e1 - e0) <= (e - e0) * len(todo):
                    todo[done]()
                    done += 1
                q = jnp.concatenate([g_s[u][d * NC + c] for c in range(NC)], axis=1)
                for a in range(2):
                    term = jnp.concatenate([kb_s[half][(2 * pair + a) * KSTRIDE + d]] * NC, axis=1) * q
                    sums[a] = term if d == 0 else sums[a] + term
                if d == DH - 1:
                    store_exp(half, 16 * pair, cols, jnp.concatenate(sums, axis=0))
            for job in todo[done:]:
                job()

            if i + AHEAD == len(steps) - 1:
                held.append(probabilities(i + AHEAD))
            elif i + AHEAD < len(steps):
                weigh_values(i + AHEAD, previous, slot)
            elif i == len(steps) - 1:
                weigh_values(i, previous, slot, held[0])

    h0 = jnp.int32(0)
    for u in range(NU):
        for job in w_jobs(h0, u) + q_jobs(h0, u):
            job()
    for half in range(2):
        for u in range(NU):
            for job in k_jobs(h0, half, u):
                job()
    lax.fori_loop(0, H, one_head, None)

    def merge_heads(b):
        cols = pl.ds(b * TB, TB)
        rows = []
        for h in range(0, H, 2):
            even, odd = ot_s[h, :, cols], ot_s[h + 1, :, cols]
            r = 1.0 / jnp.where(sub < 4, odd[0:8], even[16:24])
            re = jnp.broadcast_to(r[4:5], (8, TB))
            ro = jnp.broadcast_to(r[0:1], (8, TB))
            rows += [even[0:8] * re, even[8:16] * re, jnp.where(sub < 4, even[16:24] * re, odd[0:8] * ro),
                     odd[8:16] * ro, odd[16:24] * ro]
        return jnp.concatenate(rows, axis=0).T

    for cp in later_cp:
        cp.wait()
    for i in sorted(range(len(steps)), key=lambda i: steps[i][1]):
        weigh_values(i, H - 1, H - 1)
    o_s[...] = merge_heads(0)

    row_sums = [jnp.where(sub8 < 4, ot_s[h + 1, 0:8, pl.ds(c, L)], ot_s[h, 16:24, pl.ds(c, L)])
                for h in range(0, H, 2) for c in range(0, S, L)]
    lo = functools.reduce(jnp.minimum, [functools.reduce(jnp.minimum, row_sums[i::8]) for i in range(8)])
    hi = functools.reduce(jnp.maximum, [functools.reduce(jnp.maximum, row_sums[i::8]) for i in range(8)])
    safe = jnp.logical_and(lo >= 2.0 ** -40, hi <= 2.0 ** 64)

    @pl.when(jnp.max(jnp.where(safe, 0.0, 1.0)) > 0.5)
    def _():
        def with_true_max(h, carry):
            slab = slab_of(h)
            for u in range(NU):
                w = pltpu.bitcast(jnp.concatenate([
                    jnp.concatenate([w_tile(h, slab, u, c, i) for i in range(8)], axis=0)
                    for c in range(NC)], axis=1), BF16)

                def some_keys(c, state, w=w):
                    m, acc = state
                    keys = k_s[slab, pl.ds(pl.multiple_of(c * 128, 128), 128), :]
                    s = mm(pltpu.bitcast(keys, BF16), w)
                    top = jnp.maximum(m, jnp.max(s, axis=0, keepdims=True))
                    p = jnp.exp2(s - top).astype(BF16)
                    values = vt_s[h, :, pl.ds(pl.multiple_of(c * 256, 256), 256)]
                    return top, acc * jnp.exp2(m - top) + mm(values, p)

                start = (jnp.full((1, BQ), -jnp.inf, F32), jnp.zeros((24, BQ), F32))
                ot_s[h, :, pl.ds(u * BQ, BQ)] = lax.fori_loop(0, S // 256, some_keys, start)[1]
        lax.fori_loop(0, H, with_true_max, None)
        o_s[...] = merge_heads(0)

    b1 = b1_s[...].astype(F32).reshape(1, F)
    b2 = b2_s[...].astype(F32).reshape(1, D)
    out_cp = [pltpu.make_async_copy(out_s.at[pl.ds(b * TB, TB)], out_hbm.at[pl.ds(b * TB, TB)], out_sem.at[b])
              for b in range(NB)]

    def attention_out(b):
        o = cut(o_s[...] if b == 0 else merge_heads(b))
        ob = assemble(o, TB, D).astype(BF16)
        rest = []
        main = strassen(operands(o, TB, KS, LEFT), ro_s, "2341056x", lambda: rest.extend(
            [cut(mm(ob[:, KS:], wo_s[KS:, :KS])), cut(mm(ob, wo_s[:, KS:]))]))

        @functools.cache
        def residual(r, c):
            x = x_s[pl.ds(b * TB + r, RC), pl.ds(c, L)].astype(F32)
            return x + main(r, c) + rest[0](r, c) if c < KS else x + rest[1](r, 0)
        return residual

    def hidden(residual):
        hn = layernorm(residual)
        rest = []
        main = strassen(operands(hn, TB, KS, LEFT), r1_s, "x1432056", lambda: rest.append(
            cut(mm(assemble(lambda r, c: hn(r, KS), TB, L).astype(BF16), w1_s[KS:, :]))))

        @functools.cache
        def activation(r, c):
            a = jnp.maximum(main(r, c) + rest[0](r, c) + b1[:, c:c + L], 0.0)
            return a * a
        return activation

    def finish(b, residual, activation):
        rest = []
        main = strassen(operands(activation, TB, F, LEFT), r2_s, "0654213x", lambda: rest.append(
            cut(mm(assemble(activation, TB, F).astype(BF16), w2_s[:, KS:]))))
        for r0 in range(0, TB // 2, RC):
            for r in (r0, r0 + TB // 2):
                y = [(main(r, c) if c < KS else rest[0](r, 0)) + b2[:, c:c + L] + residual(r, c)
                     for c in range(0, D, L)]
                out_s[pl.ds(b * TB + r, RC), :] = jnp.concatenate(y, axis=1).astype(BF16)
        out_cp[b].start()

    store_right(ro_s, wo_s, KS, KS)
    store_right(r1_s, w1_s, KS, F)
    store_right(r2_s, w2_s, F, KS)
    residual, activation = {0: attention_out(0)}, {}
    for b in range(NB):
        if b + 1 < NB:
            residual[b + 1] = attention_out(b + 1)
        activation[b] = hidden(residual[b])
        if b:
            finish(b - 1, residual[b - 1], activation[b - 1])
    finish(NB - 1, residual[NB - 1], activation[NB - 1])
    for cp in out_cp:
        cp.wait()


@jax.jit
def pallas_sequential_preLN__softmax_full_mha__dense_activation_squared_relu__prompt_kernel(
    A_x: jax.Array,
    A_wqkv: jax.Array,
    A_wo: jax.Array,
    B_x: jax.Array,
    B_w1: jax.Array,
    B_b1: jax.Array,
    B_w2: jax.Array,
    B_b2: jax.Array,
):
    del B_x

    def halves(k, n):
        return pltpu.VMEM((7 * k // 4, n // 2), U32)

    scratch = [
        pltpu.VMEM((S, D), BF16), pltpu.VMEM((D, 3 * D), BF16), pltpu.VMEM((D, D), BF16),
        pltpu.VMEM((D, F), BF16), pltpu.VMEM((F, D), BF16), pltpu.VMEM((S, D), BF16),
        halves(KS, NQ), halves(KS, KS), halves(KS, F), halves(F, KS),
        pltpu.VMEM((TB, D), F32),
        pltpu.VMEM((NSL, S // 2, L), F32),
        pltpu.VMEM((H, 24, S), F32),
        pltpu.VMEM((8, L // 2, BQ), F32),
        *[pltpu.VMEM((8 * G_END, L), F32)] * NU,
        *[pltpu.VMEM((KSPARE + 1, 8, L), F32)] * 2,
        *[pltpu.VMEM((SK // 2 + 8, S), U32)] * 2,
        pltpu.VMEM((H + 1, 24, S), F32),
        pltpu.VMEM((32, BQ), F32),
        pltpu.VMEM((F,), BF16), pltpu.VMEM((D,), BF16),
        pltpu.SMEM((3,), jnp.int32),
        pltpu.SemaphoreType.DMA((7 + NB,)), pltpu.SemaphoreType.DMA((NB,)),
    ]
    hbm = pl.BlockSpec(memory_space=pl.ANY)
    out = pl.pallas_call(
        kernel,
        out_shape=jax.ShapeDtypeStruct((S, D), BF16),
        in_specs=[hbm] * 7,
        out_specs=hbm,
        scratch_shapes=scratch,
        compiler_params=pltpu.CompilerParams(vmem_limit_bytes=110 * 2 ** 20),
    )(A_x.reshape(S, D), A_wqkv, A_wo, B_w1, B_b1, B_w2, B_b2)
    return out.reshape(1, S, D)
```
